```python
import os as _os
_os.environ.setdefault("JAX_PLATFORMS", "cpu")
import jax
import jax.numpy as jnp

def _softmax(x, axis=-1):
    return jax.nn.softmax(x, axis=axis)
def _gelu(x):
    return jax.nn.gelu(x, approximate=True)
def _silu(x):
    return jax.nn.silu(x)
def _sigmoid(x):
    return jax.nn.sigmoid(x)
def _layernorm(x, axis=-1, eps=1e-5):
    m = jnp.mean(x, axis=axis, keepdims=True)
    v = jnp.var(x, axis=axis, keepdims=True)
    return (x - m) / jnp.sqrt(v + eps)
def _scatter_add(tgt, idx, src, axis=0):
    return tgt.at[idx].add(src)
def _segment_sum(src, seg, n):
    return jax.ops.segment_sum(src, seg, n)
class _Rng:
    def __init__(self, key):
        self._k = key
    def _next(self):
        self._k, sub = jax.random.split(self._k)
        return sub
    def normal(self, shape):
        return jax.random.normal(self._next(), shape, dtype=jnp.bfloat16)
    def randint(self, lo, hi, shape):
        return jax.random.randint(self._next(), shape, lo, hi, dtype=jnp.int32)
    def uniform(self, shape, lo=0.0, hi=1.0):
        return jax.random.uniform(self._next(), shape, jnp.bfloat16, lo, hi)
    def permutation(self, n):
        return jax.random.permutation(self._next(), n)


kernel_name = 'interleave_layers__linear_kernel_hedgehog__dense_activation_silu__prompt'

def setup_inputs():
    _rng = _Rng(jax.random.key(int.from_bytes(__import__("os").urandom(4), "little")))
    _w = (lambda a: (lambda t: t.astype(jnp.bfloat16) if jnp.issubdtype(t.dtype, jnp.floating) else t)(jnp.asarray(a)))
    def _A_setup():
        B, S, D, H = 1, 2048, 640, 32
        Dh = D // H
        return {
            "x": _w((lambda *s: _rng.normal(s) * 0.05)(B, S, D)),
            "wqkv": _w((lambda *s: _rng.normal(s) * 0.4)(D, 3 * D)),
            "w_phi": _w((lambda *s: _rng.normal(s) * 0.4)(H, Dh, Dh) * (Dh ** -0.5)),
            "wo": _w((lambda *s: _rng.normal(s) * 0.05)(D, D)),
        }
    _A_in = _A_setup()

    def _B_setup():
        B, S, D, F = 1, 2048, 640, 1728
        return {
            "x": _w((lambda *s: _rng.normal(s) * 0.05)(B, S, D)),
            "w1": _w((lambda *s: _rng.normal(s) * 1.6)(D, F) * (D ** -0.5)),
            "w2": _w((lambda *s: _rng.normal(s) * 1.6)(F, D) * (F ** -0.5)),
        }
    _B_in = _B_setup()

    return {
        "A_x": _A_in["x"],
        "A_wqkv": _A_in["wqkv"],
        "A_w_phi": _A_in["w_phi"],
        "A_wo": _A_in["wo"],
        "B_x": _B_in["x"],
        "B_w1": _B_in["w1"],
        "B_w2": _B_in["w2"],
    }

def reference(A_x, A_wqkv, A_w_phi, A_wo, B_x, B_w1, B_w2):
    def _A_ref(x, wqkv, w_phi, wo):
        B, S, D = x.shape
        H = 32; Dh = D // H
        qkv = (lambda x, *d: x.transpose(*d))((x @ wqkv).reshape(B, S, 3, H, Dh), 2, 0, 3, 1, 4)
        q, k, v = qkv[0], qkv[1], qkv[2]
        pq = jnp.einsum("bhsd,hdf->bhsf", q, w_phi)
        pk = jnp.einsum("bhsd,hdf->bhsf", k, w_phi)
        phi_q = jnp.concatenate([_softmax(pq, axis=-1), _softmax(-pq, axis=-1)], axis=-1)
        phi_k = jnp.concatenate([_softmax(pk, axis=-1), _softmax(-pk, axis=-1)], axis=-1)
        kv = jnp.einsum("bhsf,bhsd->bhfd", phi_k, v)
        z  = jnp.einsum("bhsf->bhf", phi_k)
        num = jnp.einsum("bhqf,bhfd->bhqd", phi_q, kv)
        den = jnp.einsum("bhqf,bhf->bhq", phi_q, z)[..., None] + 1e-6
        o = num / den
        return (lambda x, *d: x.transpose(*d))(o, 0, 2, 1, 3).reshape(B, S, D) @ wo

    def _B_ref(x, w1, w2):
        h = jnp.einsum("bsd,df->bsf", x, w1)
        h = _silu(h)
        out = jnp.einsum("bsf,fd->bsd", h, w2)
        return out

    x = A_x
    x = x + _A_ref(_layernorm(x, axis=-1), A_wqkv, A_w_phi, A_wo)
    x = x + _B_ref(_layernorm(x, axis=-1), B_w1, B_w2)
    x = x + _A_ref(_layernorm(x, axis=-1), A_wqkv, A_w_phi, A_wo)
    x = x + _B_ref(_layernorm(x, axis=-1), B_w1, B_w2)
    return x
```

```python
import contextlib

import jax
import jax.numpy as jnp
from jax import lax
import jax.experimental.pallas as pl
import jax.experimental.pallas.tpu as pltpu

S, D, H, F = 2048, 640, 32, 1728
DH = D // H

HPG = 2
LHPG = {2: 1, 4: 2, 8: 3}[HPG]
G = H // HPG
R = DH * HPG
SG = 8 // HPG
RS = DH * 8
NSG = H // 8
KVM = (R + 8 + 15) // 16 * 16
T = 512
NB = S // T
LOG2E = 1.4426950408889634
LN_EPS = 1e-5
DEN_EPS = 1e-6
PROFILE = False

_NN = (((1,), (0,)), ((), ()))
_NT = (((1,), (1,)), ((), ()))
f32 = jnp.float32
bf16 = jnp.bfloat16


def _scope(name):
    return jax.named_scope(name) if PROFILE else contextlib.nullcontext()


def _dot(a, b, dims=_NN):
    return lax.dot_general(a, b, dims, preferred_element_type=f32)


def _recip(x):
    r = pl.reciprocal(x, approx=True)
    return r * (2.0 - x * r)


def _row_feature_head(r):
    gl = jnp.zeros_like(r)
    for s in range(1, SG):
        gl = gl + (r >= s * R).astype(jnp.int32)
    rr = r - R * gl
    return rr >> LHPG, HPG * gl + (rr & (HPG - 1))


def _feature_map_rows(wphi):
    h = lax.broadcasted_iota(jnp.int32, (H, D), 0)
    c = lax.broadcasted_iota(jnp.int32, (H, D), 1)
    rel = c - DH * h
    wt = None
    for d in range(DH):
        e = (rel == d).astype(f32).astype(bf16)
        y = _dot(wphi[d], e)
        wt = y if wt is None else wt + y
    r = lax.broadcasted_iota(jnp.int32, (RS, DH), 0)
    f = lax.broadcasted_iota(jnp.int32, (RS, DH), 1)
    rep = (_row_feature_head(r)[0] == f).astype(f32).astype(bf16)
    return _dot(rep, wt.astype(bf16))


def _sel_matrix(j, wrep):
    ws = (RS * j // 128) * 128
    r = lax.broadcasted_iota(jnp.int32, (RS, 256), 0)
    c = lax.broadcasted_iota(jnp.int32, (RS, 256), 1) + ws
    f, head = _row_feature_head(r)
    lo = DH * (8 * j + head)
    if wrep is None:
        return (c == lo + f).astype(f32).astype(bf16), ws
    m = (c >= lo) & (c < lo + DH)
    return jnp.where(m, wrep[:, ws:ws + 256], 0.0).astype(bf16), ws


def _head_allreduce(v, op):
    sh = 4
    while sh >= HPG:
        v = op(v, pltpu.roll(v, sh, 0))
        sh //= 2
    return v


def _dual_softmax(p):
    t = p.shape[1]
    p3 = p.reshape(R // 8, 8, t)
    mx = _head_allreduce(jnp.max(p3, axis=0), jnp.maximum)
    mn = _head_allreduce(jnp.min(p3, axis=0), jnp.minimum)
    ep = jnp.exp2(p3 - mx[None])
    en = jnp.exp2(mn[None] - p3)
    sp = _head_allreduce(jnp.sum(ep, axis=0), jnp.add)
    sn = _head_allreduce(jnp.sum(en, axis=0), jnp.add)
    ep = ep * _recip(sp)[None]
    en = en * _recip(sn)[None]
    return jnp.concatenate([ep.reshape(R, t), en.reshape(R, t)], axis=0).astype(bf16)


def _ln(x, scale=1.0):
    m = jnp.sum(x, axis=0, keepdims=True) * (1.0 / D)
    xc = x - m
    v = jnp.sum(xc * xc, axis=0, keepdims=True) * (1.0 / D)
    r = lax.rsqrt(v + LN_EPS)
    if scale != 1.0:
        r = r * scale
    return (xc * r).astype(bf16)


def _kernel(x_hbm, wqkv_hbm, wphi_hbm, wo_hbm, w1T_hbm, w2_hbm,
            out_hbm,
            xraw, wqkv_raw, wphi_raw, wo_raw, w1T, w2_raw,
            wqT, wkvT, woT, w2T,
            xT, pqs, kvacc, kvz, obuf, xsem, wsem, osem):
    x_copies = [
        pltpu.make_async_copy(x_hbm.at[pl.ds(i * T, T)], xraw.at[i], xsem.at[i])
        for i in range(NB)
    ]
    cp_wkv = pltpu.make_async_copy(
        wqkv_hbm.at[:, pl.ds(D, 2 * D)], wqkv_raw.at[:, pl.ds(D, 2 * D)], wsem.at[0])
    cp_wq = pltpu.make_async_copy(
        wqkv_hbm.at[:, pl.ds(0, D)], wqkv_raw.at[:, pl.ds(0, D)], wsem.at[5])
    cp_wo = pltpu.make_async_copy(wo_hbm, wo_raw, wsem.at[1])
    cp_w1 = pltpu.make_async_copy(w1T_hbm, w1T, wsem.at[2])
    cp_w2 = pltpu.make_async_copy(w2_hbm, w2_raw, wsem.at[3])
    cp_wphi = pltpu.make_async_copy(wphi_hbm, wphi_raw, wsem.at[4])
    cp_wphi.start()
    cp_wkv.start()
    x_copies[0].start()

    sel_id = [_sel_matrix(j, None) for j in range(NSG)]
    with _scope("wphi_wait"):
        cp_wphi.wait()
    wrep = _feature_map_rows(wphi_raw[...])
    sel_phi = [_sel_matrix(j, wrep) for j in range(NSG)]

    def load_x(i):
        x_copies[i].wait()
        x = xraw[i].T.astype(f32)
        xT[i] = x
        return _ln(x)

    with _scope("x0"):
        xn = load_x(0)
    with _scope("wkv_wait"):
        cp_wkv.wait()
    x_copies[1].start()
    cp_wq.start()
    for j in range(NSG):
        pj, ws = sel_phi[j]
        ij, _ = sel_id[j]
        wk = _dot(pj, wqkv_raw[:, D + ws:D + ws + 256], _NT) * LOG2E
        wv = _dot(ij, wqkv_raw[:, 2 * D + ws:2 * D + ws + 256], _NT)
        wkvT[2 * j * RS:(2 * j + 1) * RS, :] = wk.astype(bf16)
        wkvT[(2 * j + 1) * RS:(2 * j + 2) * RS, :] = wv.astype(bf16)
    for c in x_copies[2:]:
        c.start()
    cp_wo.start()
    cp_w2.start()
    cp_w1.start()

    def prep_wq():
        cp_wq.wait()
        for j in range(NSG):
            pj, ws = sel_phi[j]
            wq = _dot(pj, wqkv_raw[:, ws:ws + 256], _NT) * LOG2E
            wqT[j * RS:(j + 1) * RS, :] = wq.astype(bf16)

    def prep_wo():
        cp_wo.wait()
        for j in range(NSG):
            ij, ws = sel_id[j]
            woj = _dot(ij, wo_raw[ws:ws + 256, :])
            obuf[0, j * RS:(j + 1) * RS, :] = woj.astype(bf16)
        woT[...] = obuf[0, :D, :].T

    def prep_w2(lo, hi):
        if lo == 0:
            cp_w2.wait()
        w2T[:, lo:hi] = w2_raw[lo:hi, :].T

    ones = jnp.ones((KVM - R, T), f32)

    def kv_side(xn, first):
        for j in range(NSG):
            kv = _dot(wkvT[2 * j * RS:(2 * j + 2) * RS, :], xn)
            for s in range(SG):
                g = j * SG + s
                phi = _dual_softmax(kv[s * R:(s + 1) * R])
                v = kv[RS + s * R:RS + (s + 1) * R]
                va = jnp.concatenate([v, ones], axis=0).astype(bf16)
                acc = _dot(va, phi, _NT)
                if first:
                    kvacc[g] = acc
                else:
                    kvacc[g] += acc

    def kv_finalize():
        r = lax.broadcasted_iota(jnp.int32, (KVM, 2 * R), 0)
        c = lax.broadcasted_iota(jnp.int32, (KVM, 2 * R), 1)
        m = (r & (HPG - 1)) == (c & (HPG - 1))
        for g in range(G):
            kvz[g] = jnp.where(m, kvacc[g], 0.0).astype(bf16)

    def q_proj(i, xn):
        pqs[i] = _dot(wqT[...], xn)

    def q_side(i):
        os = []
        for j in range(NSG):
            oj = []
            for s in range(SG):
                g = j * SG + s
                phi = _dual_softmax(pqs[i, g * R:(g + 1) * R, :])
                nd = _dot(kvz[g], phi)
                rden = _recip(nd[R:R + 8] + DEN_EPS)
                o = nd[:R].reshape(R // 8, 8, T) * rden[None]
                oj.append(o.reshape(R, T))
            os.append(jnp.concatenate(oj, axis=0).astype(bf16))
        o = jnp.concatenate(os, axis=0)
        return xT[i] + _dot(woT[...], o)

    def ffn(x):
        xn = _ln(x, 0.5)
        h = _dot(w1T[...], xn)
        h = (h + h * jnp.tanh(h)).astype(bf16)
        return x + _dot(w2T[...], h)

    w2_cuts = (0, 0, 896, F, F)
    for i in range(NB):
        with _scope("pass1_%d" % i):
            if i > 0:
                xn = load_x(i)
            kv_side(xn, i == 0)
            if i == 0:
                prep_wq()
            if i == 1:
                prep_wo()
            if w2_cuts[i + 1] > w2_cuts[i]:
                prep_w2(w2_cuts[i], w2_cuts[i + 1])
            q_proj(i, xn)
    cp_w1.wait()
    kv_finalize()

    for i in range(NB):
        with _scope("pass2_%d" % i):
            x = ffn(q_side(i))
            xT[i] = x
            xn = _ln(x)
            kv_side(xn, i == 0)
            q_proj(i, xn)
    kv_finalize()

    def out_copy(i, slot):
        return pltpu.make_async_copy(
            obuf.at[slot, pl.ds(0, T)], out_hbm.at[pl.ds(i * T, T)], osem.at[slot])

    for i in range(NB):
        with _scope("pass3_%d" % i):
            slot = i % 2
            x = ffn(q_side(i))
            if i >= 2:
                out_copy(i - 2, slot).wait()
            obuf[slot, :T, :] = x.astype(bf16).T
            out_copy(i, slot).start()
    with _scope("outwait"):
        for i in range(max(NB - 2, 0), NB):
            out_copy(i, i % 2).wait()


@jax.jit
def pallas_interleave_layers__linear_kernel_hedgehog__dense_activation_silu__prompt_kernel(
    A_x: jax.Array,
    A_wqkv: jax.Array,
    A_w_phi: jax.Array,
    A_wo: jax.Array,
    B_x: jax.Array,
    B_w1: jax.Array,
    B_w2: jax.Array,
):
    del B_x
    x = A_x.reshape(S, D)
    wphi = A_w_phi.transpose(1, 2, 0)
    w1T = B_w1.T

    hbm_spec = pl.BlockSpec(memory_space=pltpu.MemorySpace.HBM)
    ot = max(T, D)
    out = pl.pallas_call(
        _kernel,
        out_shape=jax.ShapeDtypeStruct((S, D), A_x.dtype),
        in_specs=[hbm_spec] * 6,
        out_specs=hbm_spec,
        scratch_shapes=[
            pltpu.VMEM((NB, T, D), bf16),
            pltpu.VMEM((D, 3 * D), bf16),
            pltpu.VMEM((DH, DH, H), bf16),
            pltpu.VMEM((D, D), bf16),
            pltpu.VMEM((F, D), bf16),
            pltpu.VMEM((F, D), bf16),
            pltpu.VMEM((D, D), bf16),
            pltpu.VMEM((2 * D, D), bf16),
            pltpu.VMEM((D, D), bf16),
            pltpu.VMEM((D, F), bf16),
            pltpu.VMEM((NB, D, T), f32),
            pltpu.VMEM((NB, D, T), f32),
            pltpu.VMEM((G, KVM, 2 * R), f32),
            pltpu.VMEM((G, KVM, 2 * R), bf16),
            pltpu.VMEM((2, ot, D), bf16),
            pltpu.SemaphoreType.DMA((NB,)),
            pltpu.SemaphoreType.DMA((6,)),
            pltpu.SemaphoreType.DMA((2,)),
        ],
        compiler_params=pltpu.CompilerParams(
            vmem_limit_bytes=100 * 1024 * 1024,
        ),
    )(x, A_wqkv, wphi, A_wo, w1T, B_w2)
    return out.reshape(1, S, D)
```

```python
import jax
import jax.numpy as jnp
from jax import lax
import jax.experimental.pallas as pl
import jax.experimental.pallas.tpu as pltpu

S, D, H, F = 2048, 640, 32, 1728
DH = D // H

HPG = 2
G = H // HPG
R = DH * HPG
SG = 8 // HPG
RS = DH * 8
NSG = H // 8
KVM = (R + 8 + 15) // 16 * 16
NT = D // 128
T = 512
NB = S // T
LOG2E = 1.4426950408889634
LN_EPS = 1e-5
DEN_EPS = 1e-6

_NN = (((1,), (0,)), ((), ()))
_NT = (((1,), (1,)), ((), ()))
f32 = jnp.float32
bf16 = jnp.bfloat16


def _dot(a, b, dims=_NN):
    return lax.dot_general(a, b, dims, preferred_element_type=f32)


def _recip(x):
    r = pl.reciprocal(x, approx=True)
    return r * (2.0 - x * r)


def _fold_constants():
    h = lax.broadcasted_iota(jnp.int32, (H, D), 0)
    c = lax.broadcasted_iota(jnp.int32, (H, D), 1)
    rel = c - DH * h
    spread = [(rel == d).astype(f32).astype(bf16) for d in range(DH)]
    r = lax.broadcasted_iota(jnp.int32, (R, DH), 0)
    f = lax.broadcasted_iota(jnp.int32, (R, DH), 1)
    rep = ((r >> 1) == f).astype(f32).astype(bf16)
    r = lax.broadcasted_iota(jnp.int32, (RS, 128), 0)
    c = lax.broadcasted_iota(jnp.int32, (RS, 128), 1)
    gl = sum((r >= k * R).astype(jnp.int32) for k in range(1, 4))
    head = 2 * gl + (r & 1)
    masks = []
    for t in range(NT):
        lo = DH * (head + 6 * t) - 128 * t
        masks.append((c >= lo) & (c < lo + DH))
    return spread, rep, masks


def _fold_operands(wphi, consts):
    spread, rep, masks = consts
    wt = None
    for d in range(DH):
        y = _dot(wphi[d], spread[d])
        wt = y if wt is None else wt + y
    wrep = _dot(rep, wt.astype(bf16))
    out = []
    for t in range(NT):
        w = wrep[:, 128 * t:128 * (t + 1)]
        w = jnp.concatenate([w] * 4, axis=0)
        out.append(jnp.where(masks[t], w, 0.0).astype(bf16))
    return out


def _fold(sel, w_ref, col0):
    parts = [_dot(sel[t], w_ref[:, col0 + 128 * t:col0 + 128 * (t + 1)], _NT)
             for t in range(NT)]
    rows = [parts[0][:3 * R]]
    for t in range(1, NT):
        rows.append(parts[t - 1][3 * R:] + parts[t][:R])
        rows.append(parts[t][R:3 * R])
    rows.append(parts[NT - 1][3 * R:])
    return (jnp.concatenate(rows, axis=0) * LOG2E).astype(bf16)


def _head_allreduce(v, op):
    sh = 4
    while sh >= HPG:
        v = op(v, pltpu.roll(v, sh, 0))
        sh //= 2
    return v


def _dual_softmax(p):
    t = p.shape[1]
    p3 = p.reshape(R // 8, 8, t)
    mx = _head_allreduce(jnp.max(p3, axis=0), jnp.maximum)
    mn = _head_allreduce(jnp.min(p3, axis=0), jnp.minimum)
    ep = jnp.exp2(p3 - mx[None])
    en = jnp.exp2(mn[None] - p3)
    sp = _head_allreduce(jnp.sum(ep, axis=0), jnp.add)
    sn = _head_allreduce(jnp.sum(en, axis=0), jnp.add)
    ep = ep * _recip(sp)[None]
    en = en * _recip(sn)[None]
    return jnp.concatenate([ep.reshape(R, t), en.reshape(R, t)], axis=0).astype(bf16)


def _ln(x, scale=1.0):
    m = jnp.sum(x, axis=0, keepdims=True) * (1.0 / D)
    xc = x - m
    v = jnp.sum(xc * xc, axis=0, keepdims=True) * (1.0 / D)
    r = lax.rsqrt(v + LN_EPS)
    if scale != 1.0:
        r = r * scale
    return (xc * r).astype(bf16)


def _kernel(x_hbm, wqkv_hbm, wphi_hbm, wo_hbm, w1T_hbm, w2_hbm,
            out_hbm,
            xraw, wqkv_raw, wphi_raw, wo_raw, w1T, w2_raw,
            wqT, wkT, wvT, woT, w2T,
            xT, pqs, kvacc, kvz, obuf, xsem, wsem, osem):
    x_copies = [
        pltpu.make_async_copy(x_hbm.at[pl.ds(i * T, T)], xraw.at[i], xsem.at[i])
        for i in range(NB)
    ]
    cp_wq, cp_wk, cp_wv = [
        pltpu.make_async_copy(wqkv_hbm.at[:, pl.ds(k * D, D)],
                              wqkv_raw.at[:, pl.ds(k * D, D)], wsem.at[4 + k])
        for k in range(3)
    ]
    cp_wo = pltpu.make_async_copy(wo_hbm, wo_raw, wsem.at[0])
    cp_w1 = pltpu.make_async_copy(w1T_hbm, w1T, wsem.at[1])
    cp_w2 = pltpu.make_async_copy(w2_hbm, w2_raw, wsem.at[2])
    cp_wphi = pltpu.make_async_copy(wphi_hbm, wphi_raw, wsem.at[3])
    cp_wphi.start()
    x_copies[0].start()
    cp_wk.start()
    cp_wv.start()
    cp_wq.start()
    x_copies[1].start()

    fold_consts = _fold_constants()
    cp_wphi.wait()
    x_copies[0].wait()
    sel = _fold_operands(wphi_raw[...], fold_consts)

    ones = jnp.ones((KVM - R, T), f32)
    low_half = lax.broadcasted_iota(jnp.int32, (8, T), 0) < 4
    QCUT = (0, RS, 2 * RS, 3 * RS, D)
    OCUT = (0, 256, 512, D)
    FCUT = (0, 512, 1024, 1536, F)

    class Blk:
        def __init__(self, i):
            self.i = i
            self.o, self.x1, self.h, self.x2 = [], [], [], []
            self.xn = self.xn1 = None
            self.phik = {}

    def load_x(b):
        x = xraw[b.i].T.astype(f32)
        xT[b.i] = x
        b.xn = _ln(x)

    def k_chunk(b, j):
        pk = _dot(wkT[j * RS:(j + 1) * RS, :], b.xn)
        b.phik[j] = [_dual_softmax(pk[s * R:(s + 1) * R]) for s in range(SG)]

    def kv_chunk(b, j):
        if j not in b.phik:
            k_chunk(b, j)
        vj = _dot(wvT[j * RS:(j + 1) * RS, :], b.xn)
        for s in range(SG):
            g = j * SG + s
            phi = b.phik[j][s]
            v = vj[s * R:(s + 1) * R]
            va = jnp.concatenate([v, ones], axis=0).astype(bf16)
            acc = _dot(va, phi, _NT)
            if b.i == 0:
                kvacc[g] = acc
            else:
                kvacc[g] += acc

    def kv_finalize():
        r = lax.broadcasted_iota(jnp.int32, (KVM, 2 * R), 0)
        c = lax.broadcasted_iota(jnp.int32, (KVM, 2 * R), 1)
        rh = jnp.where(r < R, (r >= DH).astype(jnp.int32),
                       (r >= R + 4).astype(jnp.int32))
        m = rh == (c & 1)
        for g in range(G):
            kvz[g] = jnp.where(m, kvacc[g], 0.0).astype(bf16)

    def qp_chunk(b, j):
        rows = slice(j * RS, (j + 1) * RS)
        pqs[b.i, rows, :] = _dot(wqT[rows, :], b.xn)

    def qsn_chunk(b, j):
        oj = []
        for s in range(SG):
            g = j * SG + s
            phi = _dual_softmax(pqs[b.i, g * R:(g + 1) * R, :])
            nd = _dot(kvz[g], phi)
            rab = _recip(nd[R:R + 8] + DEN_EPS)
            rba = pltpu.roll(rab, 4, 0)
            raa = jnp.where(low_half, rab, rba)
            rbb = jnp.where(low_half, rba, rab)
            o = nd[:R] * jnp.concatenate([raa, raa, rab, rbb, rbb], axis=0)
            oj.append(o)
        b.o += oj

    def wo_chunk(b, c):
        rows = slice(c * RS, (c + 1) * RS)
        o = jnp.concatenate(b.o, axis=0).astype(bf16)
        b.x1.append(xT[b.i, rows, :] + _dot(woT[rows, :], o))

    def ln1(b):
        b.xn1 = _ln(jnp.concatenate(b.x1, axis=0), 0.5)

    def f1_chunk(b, c):
        h = _dot(w1T[FCUT[c]:FCUT[c + 1], :], b.xn1)
        b.h.append(h + h * jnp.tanh(h))

    def f2_chunk(b, c, cuts=QCUT, out=False):
        lo, hi = cuts[c], cuts[c + 1]
        h = jnp.concatenate(b.h, axis=0).astype(bf16)
        x2 = jnp.concatenate(b.x1, axis=0)[lo:hi] + _dot(w2T[lo:hi, :], h)
        if out:
            store_out(b, c, x2)
        else:
            b.x2.append(x2)

    def ln2(b):
        x = jnp.concatenate(b.x2, axis=0)
        xT[b.i] = x
        b.xn = _ln(x)

    def prep_wq():
        wqT[...] = _fold(sel, wqkv_raw, 0)

    def prep_wo():
        woT[...] = wo_raw[...].T

    def prep_w2(lo, hi):
        w2T[:, lo:hi] = w2_raw[lo:hi, :].T

    def out_copy(i):
        return pltpu.make_async_copy(
            obuf.at[i], out_hbm.at[pl.ds(i * T, T)], osem.at[i])

    def last_copy(c):
        cols = pl.ds(OCUT[c], OCUT[c + 1] - OCUT[c])
        return pltpu.make_async_copy(
            obuf.at[NB - 1, :, cols], out_hbm.at[pl.ds((NB - 1) * T, T), cols],
            osem.at[NB - 1 + c])

    def store_out(b, c, x2):
        obuf[b.i, :, OCUT[c]:OCUT[c + 1]] = x2.astype(bf16).T
        if b.i == NB - 1:
            last_copy(c).start()
        elif c == len(OCUT) - 2:
            out_copy(b.i).start()

    p1 = [Blk(i) for i in range(NB)]
    load_x(p1[0])
    cp_wk.wait()
    wkT[...] = _fold(sel, wqkv_raw, D)
    for j in range(NSG):
        k_chunk(p1[0], j)
    cp_wv.wait()
    wvT[...] = wqkv_raw[:, 2 * D:].T

    for i in range(NB):
        b = p1[i]
        for j in range(NSG):
            kv_chunk(b, j)
            if j == 1 and i == 0:
                cp_wq.wait()
                x_copies[1].wait()
                for c in x_copies[2:]:
                    c.start()
                prep_wq()
            if j == 1 and i == 1:
                for c in x_copies[2:]:
                    c.wait()
                for c in (cp_wo, cp_w2, cp_w1):
                    c.start()
            if j == (2 if i == 0 else 1) and i + 1 < NB:
                load_x(p1[i + 1])
            if i > 0:
                qp_chunk(p1[i - 1], j)
        if i == NB - 1:
            for c in (cp_wo, cp_w2, cp_w1):
                c.wait()
            prep_wo()

    p2 = [Blk(i) for i in range(NB)]
    for i in range(NB):
        b = p2[i]
        a = p2[i - 1] if i > 0 else None
        for j in range(NSG):
            if a is None:
                qp_chunk(p1[NB - 1], j)
                if j == 0:
                    kv_finalize()
            qsn_chunk(b, j)
            if a is not None:
                f2_chunk(a, j)
        if a is not None:
            ln2(a)
        for c in range(NSG):
            wo_chunk(b, c)
        if a is not None:
            kv_chunk(a, 0)
        ln1(b)
        for c in range(NSG):
            f1_chunk(b, c)
            if a is None:
                prep_w2(FCUT[c], FCUT[c + 1])
            if a is not None:
                if c + 1 < NSG:
                    kv_chunk(a, c + 1)
                qp_chunk(a, c)
    a = p2[NB - 1]
    for c in range(NSG):
        f2_chunk(a, c)
    ln2(a)
    for j in range(NSG):
        kv_chunk(a, j)

    p3 = [Blk(i) for i in range(NB)]
    for i in range(NB):
        b = p3[i]
        a = p3[i - 1] if i > 0 else None
        for j in range(NSG):
            if a is None:
                qp_chunk(p2[NB - 1], j)
                if j == 0:
                    kv_finalize()
            qsn_chunk(b, j)
            if a is not None and j % 2 == 0:
                f2_chunk(a, j // 2, OCUT, True)
        for c in range(NSG):
            wo_chunk(b, c)
        ln1(b)
        if a is not None:
            f2_chunk(a, 2, OCUT, True)
        for c in range(NSG):
            f1_chunk(b, c)
    a = p3[NB - 1]
    for c in range(len(OCUT) - 1):
        f2_chunk(a, c, OCUT, True)
    for i in range(NB - 1):
        out_copy(i).wait()
    for c in range(len(OCUT) - 1):
        last_copy(c).wait()


@jax.jit
def pallas_interleave_layers__linear_kernel_hedgehog__dense_activation_silu__prompt_kernel(
    A_x: jax.Array,
    A_wqkv: jax.Array,
    A_w_phi: jax.Array,
    A_wo: jax.Array,
    B_x: jax.Array,
    B_w1: jax.Array,
    B_w2: jax.Array,
):
    del B_x
    x = A_x.reshape(S, D)
    wphi = A_w_phi.transpose(1, 2, 0)
    w1T = B_w1.T

    hbm_spec = pl.BlockSpec(memory_space=pltpu.MemorySpace.HBM)
    out = pl.pallas_call(
        _kernel,
        out_shape=jax.ShapeDtypeStruct((S, D), A_x.dtype),
        in_specs=[hbm_spec] * 6,
        out_specs=hbm_spec,
        scratch_shapes=[
            pltpu.VMEM((NB, T, D), bf16),
            pltpu.VMEM((D, 3 * D), bf16),
            pltpu.VMEM((DH, DH, H), bf16),
            pltpu.VMEM((D, D), bf16),
            pltpu.VMEM((F, D), bf16),
            pltpu.VMEM((F, D), bf16),
            pltpu.VMEM((D, D), bf16),
            pltpu.VMEM((D, D), bf16),
            pltpu.VMEM((D, D), bf16),
            pltpu.VMEM((D, D), bf16),
            pltpu.VMEM((D, F), bf16),
            pltpu.VMEM((NB, D, T), f32),
            pltpu.VMEM((NB, D, T), f32),
            pltpu.VMEM((G, KVM, 2 * R), f32),
            pltpu.VMEM((G, KVM, 2 * R), bf16),
            pltpu.VMEM((NB, T, D), bf16),
            pltpu.SemaphoreType.DMA((NB,)),
            pltpu.SemaphoreType.DMA((7,)),
            pltpu.SemaphoreType.DMA((NB + 2,)),
        ],
        compiler_params=pltpu.CompilerParams(
            vmem_limit_bytes=100 * 1024 * 1024,
            flags={"XLA_TPU_FORCE_LP_LLO_SCHEDULER": True},
        ),
    )(x, A_wqkv, wphi, A_wo, w1T, B_w2)
    return out.reshape(1, S, D)
```
